```python
import jax
import jax.numpy as jnp

def _softmax(x, axis=-1):
    return jax.nn.softmax(x, axis=axis)

def _gelu(x):
    return jax.nn.gelu(x, approximate=True)

def _silu(x):
    return jax.nn.silu(x)

def _sigmoid(x):
    return jax.nn.sigmoid(x)

def _layernorm(x, axis=-1, eps=1e-05):
    m = jnp.mean(x, axis=axis, keepdims=True)
    v = jnp.var(x, axis=axis, keepdims=True)
    return (x - m) / jnp.sqrt(v + eps)

def _scatter_add(tgt, idx, src, axis=0):
    return tgt.at[idx].add(src)

def _segment_sum(src, seg, n):
    return jax.ops.segment_sum(src, seg, n)

class _Rng:

    def __init__(self, key):
        self._k = key

    def _next(self):
        self._k, sub = jax.random.split(self._k)
        return sub

    def normal(self, shape):
        return jax.random.normal(self._next(), shape, dtype=jnp.bfloat16)

    def randint(self, lo, hi, shape):
        return jax.random.randint(self._next(), shape, lo, hi, dtype=jnp.int32)

    def uniform(self, shape, lo=0.0, hi=1.0):
        return jax.random.uniform(self._next(), shape, jnp.bfloat16, lo, hi)

    def permutation(self, n):
        return jax.random.permutation(self._next(), n)
kernel_name = 'gated_mix__softmax_full_mha__memory_aug_recurrent_mem_tr__prompt'

def setup_inputs():
    _rng = _Rng(jax.random.key(int.from_bytes(__import__("os").urandom(4), "little")))
    _w = lambda a: (lambda t: t.astype(jnp.bfloat16) if jnp.issubdtype(t.dtype, jnp.floating) else t)(jnp.asarray(a))

    def _A_setup():
        B, S, D = (1, 2048, 1024)
        return {'x': _w((lambda *s: _rng.normal(s) * 0.05)(B, S, D)), 'wqkv': _w((lambda *s: _rng.normal(s) * 0.05)(D, 3 * D)), 'wo': _w((lambda *s: _rng.normal(s) * 0.05)(D, D))}
    _A_in = _A_setup()

    def _B_setup():
        B, S, Dm = (1, 2048, 1024)
        H, Dh = (32, 128)
        M, seg = (8, 32)
        seg = min(seg, S)
        S = S // seg * seg
        return {'x': _w((lambda *s: _rng.normal(s) * 0.05)(B, S, Dm)), 'mem0': _w((lambda *s: _rng.normal(s) * 0.05)(B, M, Dm)), 'Wq': _w((lambda *s: _rng.normal(s) * 0.05)(Dm, H, Dh) * Dm ** (-0.5)), 'Wk': _w((lambda *s: _rng.normal(s) * 0.05)(Dm, H, Dh) * Dm ** (-0.5)), 'Wv': _w((lambda *s: _rng.normal(s) * 0.05)(Dm, H, Dh) * Dm ** (-0.5)), 'Wo': _w((lambda *s: _rng.normal(s) * 0.05)(H, Dh, Dm) * (H * Dh) ** (-0.5)), 'seg_len': seg}
    _B_in = _B_setup()
    return {'A_x': _A_in['x'], 'A_wqkv': _A_in['wqkv'], 'A_wo': _A_in['wo'], 'B_x': _B_in['x'], 'B_mem0': _B_in['mem0'], 'B_Wq': _B_in['Wq'], 'B_Wk': _B_in['Wk'], 'B_Wv': _B_in['Wv'], 'B_Wo': _B_in['Wo'], 'B_seg_len': _B_in['seg_len'], 'gate_w': _w((lambda *s: _rng.normal(s) * 0.05)(1024))}

def reference(A_x, A_wqkv, A_wo, B_x, B_mem0, B_Wq, B_Wk, B_Wv, B_Wo, B_seg_len, gate_w):

    def _A_ref(x, wqkv, wo):
        B, S, D = x.shape
        H = 32
        Dh = D // H
        qkv = (lambda x, *d: x.transpose(*d))((x @ wqkv).reshape(B, S, 3, H, Dh), 2, 0, 3, 1, 4)
        q, k, v = (qkv[0], qkv[1], qkv[2])
        scale = Dh ** (-0.5)
        scores = jnp.einsum('bhqd,bhkd->bhqk', q, k) * scale
        p = _softmax(scores, axis=-1)
        o = jnp.einsum('bhqk,bhkd->bhqd', p, v)
        return (lambda x, *d: x.transpose(*d))(o, 0, 2, 1, 3).reshape(B, S, D) @ wo

    def _B_ref(x, mem0, Wq, Wk, Wv, Wo, seg_len):
        B, S, Dm = x.shape
        H, Dh = (Wq.shape[1], Wq.shape[2])
        M = mem0.shape[1]
        scale = Dh ** (-0.5)
        n_seg = S // seg_len
        L = M + seg_len
        idx = jnp.arange(L)
        mask = (idx[:, None] < M) | (idx[:, None] >= idx[None, :])
        mem = mem0
        outs = []
        for s in range(n_seg):
            xs = x[:, s * seg_len:(s + 1) * seg_len, :].copy()
            h = jnp.concatenate([mem, xs], axis=1)
            q = jnp.einsum('btd,dhe->bhte', h, Wq)
            k = jnp.einsum('btd,dhe->bhte', h, Wk)
            v = jnp.einsum('btd,dhe->bhte', h, Wv)
            scores = jnp.einsum('bhqe,bhke->bhqk', q, k) * scale
            scores = jnp.where(mask[None, None], scores, -1000000000.0)
            p = _softmax(scores, axis=-1)
            o = jnp.einsum('bhqk,bhke->bhqe', p, v)
            o = jnp.einsum('bhte,hed->btd', o, Wo)
            mem = o[:, :M, :].copy()
            outs.append(o[:, M:, :])
        return jnp.concatenate(outs, axis=1)
    x = A_x
    g = _sigmoid((x * gate_w).sum(-1, keepdims=True))
    a = _A_ref(x, A_wqkv, A_wo)
    b = _B_ref(x, B_mem0, B_Wq, B_Wk, B_Wv, B_Wo, B_seg_len)
    return g * a + (1 - g) * b
```

```python
import functools

import jax
import jax.numpy as jnp
import numpy as np
from jax import lax
from jax.experimental import pallas as pl
from jax.experimental.pallas import tpu as pltpu

BF16 = jnp.bfloat16
F32 = jnp.float32
U32 = jnp.uint32
LOG2E = float(np.log2(np.e))
NT_DIMS = (((1,), (1,)), ((), ()))

TQ = 512
CN = 512
CK = 128
HA = 32
GB = 4


def _b16(words):
    return pltpu.bitcast(words, BF16)


def _words(x):
    return pltpu.bitcast(x, U32)


def _kernel(
    x_hbm, wqkv_hbm, wo_hbm, mem0_ref, wq_hbm, wk_hbm, wv_hbm, wob_hbm, gate_ref,
    out_hbm,
    x_u, wqkv_u, wo_u, wob_u, wq_st, wk_st, wv_st, wq_u, wk_u, wv_u,
    k_u, qt_u, vt_u, s_scr, ot_scr, l_scr, oa_u, out_v,
    sem_x, sem_w, sem_b, sem_o,
    *, seg,
):
    S2, D = x_u.shape
    S = 2 * S2
    DA = D // HA
    NQ = S // TQ
    NGA = D // 128
    HPG = 128 // DA
    NC = S // CK
    NCB = D // CN
    HB, _, DB = wq_u.shape
    M = mem0_ref.shape[1]
    L = M + seg
    NS = S // seg

    def x_copy(i):
        rows = pl.ds(i * (TQ // 2), TQ // 2)
        return pltpu.make_async_copy(
            x_hbm.bitcast(U32).at[rows], x_u.at[rows], sem_x.at[i])

    def w_copy(j):
        return pltpu.make_async_copy(
            wqkv_hbm.bitcast(U32).at[:, pl.ds(j * CN, CN)], wqkv_u.at[j], sem_w.at[j])

    late_copies = [
        pltpu.make_async_copy(src.bitcast(U32), dst, sem_b.at[n])
        for n, (src, dst) in enumerate((
            (wq_hbm, wq_st), (wk_hbm, wk_st), (wv_hbm, wv_st),
            (wob_hbm, wob_u), (wo_hbm, wo_u)))
    ]
    x_copy(0).start()
    for j in range(3 * NCB):
        w_copy(j).start()
    for i in range(1, NQ):
        x_copy(i).start()
    for cp in late_copies:
        cp.start()

    qscale = (DA ** -0.5) * LOG2E

    def proj_body(i, carry):
        x_copy(i).wait()
        r0 = pl.multiple_of(i * (TQ // 2), TQ // 2)
        for j in range(3 * NCB):
            @pl.when(i == 0)
            def _():
                w_copy(j).wait()

            r = jnp.dot(_b16(x_u[pl.ds(r0, TQ // 2), :]), _b16(wqkv_u[j]),
                        preferred_element_type=F32)
            which, jb = divmod(j, NCB)
            rows = slice(jb * (CN // 2), (jb + 1) * (CN // 2))
            if which == 0:
                qt_u[i, rows, :] = _words((r * qscale).astype(BF16).T)
            elif which == 1:
                rb = _words(r.astype(BF16))
                for t in range(CN // 128):
                    k_u[jb * (CN // 128) + t, pl.ds(r0, TQ // 2), :] = (
                        rb[:, t * 128:(t + 1) * 128])
            else:
                vt_u[i, rows, :] = _words(r.astype(BF16).T)
        return carry

    lax.fori_loop(0, NQ, proj_body, 0)

    for cp in late_copies:
        cp.wait()

    def masked_qt(g, qb, hh):
        r0 = pl.multiple_of(g * 64 + hh * (DA // 2), DA // 2)
        parts = []
        if hh > 0:
            parts.append(jnp.zeros((hh * (DA // 2), TQ), U32))
        parts.append(qt_u[qb, pl.ds(r0, DA // 2), :])
        if hh < HPG - 1:
            parts.append(jnp.zeros(((HPG - 1 - hh) * (DA // 2), TQ), U32))
        return _b16(jnp.concatenate(parts, axis=0))

    def qk_chunk(item, c, slot, m8):
        g, qb, hh = item
        s = jnp.dot(_b16(k_u[g, c * (CK // 2):(c + 1) * (CK // 2), :]),
                    masked_qt(g, qb, hh), preferred_element_type=F32)
        s_scr[slot, c * CK:(c + 1) * CK, :] = s
        for r in range(CK // 8):
            sr = s[r * 8:(r + 1) * 8]
            m8 = sr if m8 is None else jnp.maximum(m8, sr)
        return m8, s

    def attend(cur, nxt, slot, m8, never):
        g, _, hh = cur
        mb = jnp.broadcast_to(jnp.max(m8, axis=0, keepdims=True), (8, TQ))
        v0 = pl.multiple_of(g * 64 + hh * (DA // 2), DA // 2)
        m_next = l8 = acc = prev = None
        for c in range(NC):
            m_next, s_next = qk_chunk(nxt, c, 1 - slot, m_next)
            ps = [None] * (CK // 8)
            mc = mb
            for r in reversed(range(CK // 8)):
                n = CK // 8 - 1 - r
                if prev is not None and n % 2 == 0:
                    mc = jnp.where(never, prev[n * 8:(n + 1) * 8], mb)
                p = jnp.exp2(s_scr[slot, c * CK + r * 8:c * CK + (r + 1) * 8, :] - mc)
                ps[r] = p
                l8 = p if l8 is None else l8 + p
            kb, kt = divmod(c * CK, TQ)
            vt = _b16(vt_u[kb, pl.ds(v0, DA // 2), kt:kt + CK])
            oc = jnp.dot(vt, jnp.concatenate(ps, axis=0).astype(BF16),
                         preferred_element_type=F32)
            acc = oc if acc is None else acc + oc
            prev = s_next
        return m_next, acc, l8

    def flush(g, qb):
        o = ot_scr[...].astype(BF16).T
        oa_u[g, pl.ds(pl.multiple_of(qb * (TQ // 2), TQ // 2), TQ // 2), :] = _words(o)

    NI = NGA * NQ
    DCH = D // NI

    def relayout(it):
        for st, dst in ((wq_st, wq_u), (wk_st, wk_u), (wv_st, wv_u)):
            n = DCH * (HB // 2)
            blk = st.at[pl.ds(pl.multiple_of(it * n, n), n), :]
            for half in range(DCH // 16):
                rows = pl.ds(pl.multiple_of(it * (DCH // 2) + half * 8, 8), 8)
                for j in range(HB // 2):
                    a = blk[pl.ds(half * 16 * (HB // 2) + j, 16, stride=HB // 2), :]
                    lo = pltpu.bitcast(a << 16, F32).astype(BF16)
                    hi = pltpu.bitcast(a & np.uint32(0xFFFF0000), F32).astype(BF16)
                    dst[2 * j, rows, :] = _words(lo)
                    dst[2 * j + 1, rows, :] = _words(hi)

    m8 = None
    for c in range(NC):
        m8, _ = qk_chunk((0, 0, 0), c, 0, m8)
    ot_scr[...] = jnp.zeros(ot_scr.shape, F32)

    def attn_body(it, m8):
        g, qb = it // NQ, it % NQ
        itn = jnp.minimum(it + 1, NI - 1)
        itp = jnp.maximum(it - 1, 0)
        never = jnp.full((8, TQ), it, jnp.int32) < 0
        flush(itp // NQ, itp % NQ)
        relayout(it)
        for hh in range(HPG):
            nxt = (g, qb, hh + 1) if hh + 1 < HPG else (itn // NQ, itn % NQ, 0)
            m8, acc, l8 = attend((g, qb, hh), nxt, hh % 2, m8, never)
            ot_scr[hh * DA:(hh + 1) * DA, :] = acc / jnp.sum(l8, axis=0, keepdims=True)
        return m8

    lax.fori_loop(0, NI, attn_body, m8)
    flush(NGA - 1, NQ - 1)

    row = lax.broadcasted_iota(jnp.int32, (L, L), 0)
    col = lax.broadcasted_iota(jnp.int32, (L, L), 1)
    mask = (row < M) | (row >= col)
    scale = DB ** -0.5
    NG = HB // GB

    def out_copy(s):
        rows = pl.ds(pl.multiple_of(s * seg, seg), seg)
        return pltpu.make_async_copy(out_v.at[rows], out_hbm.at[0, rows], sem_o)

    def wcat(ref, g):
        return jnp.concatenate([_b16(ref[g * GB + i]) for i in range(GB)], axis=1)

    def seg_body(s, mem):
        @pl.when(s > 0)
        def _():
            out_copy(s - 1).start()

        r0 = pl.multiple_of(s * (seg // 2), seg // 2)
        xs = _b16(x_u[pl.ds(r0, seg // 2), :]).astype(F32)
        h = jnp.concatenate([mem, xs], axis=0)
        Q, K, V, P, O = {}, {}, {}, {}, {}
        acc = [None]

        def proj(dst, ref, g):
            dst[g] = jnp.dot(h, wcat(ref, g), preferred_element_type=F32)

        def scores(g):
            q, k = Q.pop(g), K.pop(g)
            P[g] = []
            for i in range(GB):
                sl = slice(i * DB, (i + 1) * DB)
                sc = lax.dot_general(q[:, sl], k[:, sl].astype(BF16), NT_DIMS,
                                     preferred_element_type=F32) * scale
                sc = jnp.where(mask, sc, -1000000000.0)
                e = jnp.exp(sc - jnp.max(sc, axis=-1, keepdims=True))
                P[g].append((e, jnp.sum(e, axis=-1, keepdims=True)))

        def mix(g):
            v, ps = V.pop(g), P.pop(g)
            outs = []
            for i in range(GB):
                e, l = ps[i]
                o = jnp.dot(e, v[:, i * DB:(i + 1) * DB].astype(BF16),
                            preferred_element_type=F32)
                outs.append(o / l)
            O[g] = jnp.concatenate(outs, axis=1)

        def outp(g):
            n = GB * DB // 2
            r = jnp.dot(O.pop(g), _b16(wob_u[g * n:(g + 1) * n, :]),
                        preferred_element_type=F32)
            acc[0] = r if acc[0] is None else acc[0] + r

        for t in range(NG + 1):
            if t < NG:
                proj(Q, wq_u, t)
                proj(K, wk_u, t)
            else:
                proj(V, wv_u, 0)
            if t >= 1:
                scores(t - 1)
        lag = 3
        for t in range(1, NG + lag):
            if t < NG:
                proj(V, wv_u, t)
            if t - 1 < NG:
                mix(t - 1)
            if t >= lag:
                outp(t - lag)

        oa = jnp.concatenate(
            [_b16(oa_u[g, pl.ds(r0, seg // 2), :]) for g in range(NGA)], axis=1)
        a = jnp.dot(oa, _b16(wo_u[...]), preferred_element_type=F32)
        gate = jax.nn.sigmoid(
            jnp.sum(xs * gate_ref[...].astype(F32), axis=-1, keepdims=True))
        res = gate * a + (1.0 - gate) * acc[0][M:]
        out_v[pl.ds(pl.multiple_of(s * seg, seg), seg), :] = res.astype(BF16)
        return acc[0][:M].astype(BF16).astype(F32)

    lax.fori_loop(0, NS, seg_body, mem0_ref[0].astype(F32))
    out_copy(NS - 1).start()
    pltpu.make_async_copy(out_v, out_hbm.at[0], sem_o).wait()


@functools.partial(jax.jit, static_argnames=("B_seg_len",))
def pallas_gated_mix__softmax_full_mha__memory_aug_recurrent_mem_tr__prompt_kernel(
    A_x: jax.Array,
    A_wqkv: jax.Array,
    A_wo: jax.Array,
    B_x: jax.Array,
    B_mem0: jax.Array,
    B_Wq: jax.Array,
    B_Wk: jax.Array,
    B_Wv: jax.Array,
    B_Wo: jax.Array,
    B_seg_len: int,
    gate_w: jax.Array,
):
    del B_x
    B, S, D = A_x.shape
    _, HB, DB = B_Wq.shape
    seg = int(B_seg_len)
    assert B == 1 and S % TQ == 0 and D % CN == 0 and S % seg == 0 and seg % 16 == 0
    assert DB == 128 and HB % GB == 0 and B_mem0.shape[1] % 8 == 0

    hbm = pl.BlockSpec(memory_space=pl.ANY)
    vmem = pl.BlockSpec(memory_space=pltpu.VMEM)
    stage = pltpu.VMEM((D * HB // 2, DB), U32)
    per_head = pltpu.VMEM((HB, D // 2, DB), U32)
    scratch = [
        pltpu.VMEM((S // 2, D), U32),
        pltpu.VMEM((3 * D // CN, D // 2, CN), U32),
        pltpu.VMEM((D // 2, D), U32),
        pltpu.VMEM((HB * DB // 2, D), U32),
        stage, stage, stage,
        per_head, per_head, per_head,
        pltpu.VMEM((D // 128, S // 2, 128), U32),
        pltpu.VMEM((S // TQ, D // 2, TQ), U32),
        pltpu.VMEM((S // TQ, D // 2, TQ), U32),
        pltpu.VMEM((2, S, TQ), F32),
        pltpu.VMEM((128, TQ), F32),
        pltpu.VMEM((8, TQ), F32),
        pltpu.VMEM((D // 128, S // 2, 128), U32),
        pltpu.VMEM((S, D), BF16),
        pltpu.SemaphoreType.DMA((S // TQ,)),
        pltpu.SemaphoreType.DMA((3 * D // CN,)),
        pltpu.SemaphoreType.DMA((5,)),
        pltpu.SemaphoreType.DMA,
    ]
    return pl.pallas_call(
        functools.partial(_kernel, seg=seg),
        out_shape=jax.ShapeDtypeStruct((B, S, D), A_x.dtype),
        in_specs=[hbm, hbm, hbm, vmem, hbm, hbm, hbm, hbm, vmem],
        out_specs=hbm,
        scratch_shapes=scratch,
        compiler_params=pltpu.CompilerParams(vmem_limit_bytes=120 * 2**20),
    )(
        A_x.reshape(S, D), A_wqkv, A_wo, B_mem0,
        B_Wq.reshape(D * HB, DB), B_Wk.reshape(D * HB, DB), B_Wv.reshape(D * HB, DB),
        B_Wo.reshape(HB * DB, D), gate_w.reshape(1, D),
    )
```

```python
import functools

import jax
import jax.numpy as jnp
import numpy as np
from jax import lax
from jax.experimental import pallas as pl
from jax.experimental.pallas import tpu as pltpu

BF16 = jnp.bfloat16
F32 = jnp.float32
U32 = jnp.uint32
LOG2E = float(np.log2(np.e))
NT_DIMS = (((1,), (1,)), ((), ()))

TQ = 512
CN = 512
CK = 128
HA = 32
GB = 4
SKEW = 1
FLUSH_AT = 4
DEPLAG = 1
DEPEND = 2
DEPMIN = 0
FINE = 2
DEPMUL = 16


def _b16(words):
    return pltpu.bitcast(words, BF16)


def _words(x):
    return pltpu.bitcast(x, U32)


def _kernel(
    x_hbm, wqkv_hbm, wo_hbm, mem0_ref, wq_hbm, wk_hbm, wv_hbm, wob_hbm, gate_ref,
    out_hbm,
    x_u, wqkv_u, wo_u, wob_u, w_st, wq_u, wk_u, wv_u,
    k_u, qt_u, vt_u, s_scr, ot_scr, l_scr, oa_u, out_v,
    sem_x, sem_w, sem_b, sem_o,
    *, seg,
):
    S2, D = x_u.shape
    S = 2 * S2
    DA = D // HA
    NQ = S // TQ
    NGA = D // 128
    HPG = 128 // DA
    NC = S // CK
    NCB = D // CN
    HB, _, DB = wq_u.shape
    M = mem0_ref.shape[1]
    L = M + seg
    NS = S // seg

    def x_copy(i):
        rows = pl.ds(i * (TQ // 2), TQ // 2)
        return pltpu.make_async_copy(
            x_hbm.bitcast(U32).at[rows], x_u.at[rows], sem_x.at[i])

    def w_copy(j):
        return pltpu.make_async_copy(
            wqkv_hbm.bitcast(U32).at[:, pl.ds(j * CN, CN)], wqkv_u.at[j], sem_w.at[j])

    NST = D * HB // 2
    late_copies = [
        pltpu.make_async_copy(src.bitcast(U32), dst, sem_b.at[n])
        for n, (src, dst) in enumerate((
            (wq_hbm, w_st.at[pl.ds(0, NST)]), (wk_hbm, w_st.at[pl.ds(NST, NST)]),
            (wv_hbm, w_st.at[pl.ds(2 * NST, NST)]), (wob_hbm, wob_u), (wo_hbm, wo_u)))
    ]
    x_copy(0).start()
    for j in range(3 * NCB):
        w_copy(j).start()
    for i in range(1, NQ):
        x_copy(i).start()
    for cp in late_copies:
        cp.start()

    qscale = (DA ** -0.5) * LOG2E

    def proj_rows(i, first):
        x_copy(i).wait()
        r0 = i * (TQ // 2) if first else pl.multiple_of(i * (TQ // 2), TQ // 2)
        for j in range(3 * NCB):
            if first:
                w_copy(j).wait()
            r = jnp.dot(_b16(x_u[pl.ds(r0, TQ // 2), :]), _b16(wqkv_u[j]),
                        preferred_element_type=F32)
            which, jb = divmod(j, NCB)
            rows = slice(jb * (CN // 2), (jb + 1) * (CN // 2))
            if which == 0:
                qt_u[i, rows, :] = _words((r * qscale).astype(BF16).T)
            elif which == 1:
                rb = _words(r.astype(BF16))
                for t in range(CN // 128):
                    k_u[jb * (CN // 128) + t, pl.ds(r0, TQ // 2), :] = (
                        rb[:, t * 128:(t + 1) * 128])
            else:
                vt_u[i, rows, :] = _words(r.astype(BF16).T)

    proj_rows(0, True)

    @pl.loop(1, NQ)
    def _(i):
        proj_rows(i, False)

    for cp in late_copies:
        cp.wait()

    def masked_qt(g, qb, hh):
        r0 = pl.multiple_of(g * 64 + hh * (DA // 2), DA // 2)
        parts = []
        if hh > 0:
            parts.append(jnp.zeros((hh * (DA // 2), TQ), U32))
        parts.append(qt_u[qb, pl.ds(r0, DA // 2), :])
        if hh < HPG - 1:
            parts.append(jnp.zeros(((HPG - 1 - hh) * (DA // 2), TQ), U32))
        return _b16(jnp.concatenate(parts, axis=0))

    def qk_chunk(item, c, slot, m8):
        g, qb, hh = item
        s = jnp.dot(_b16(k_u[g, c * (CK // 2):(c + 1) * (CK // 2), :]),
                    masked_qt(g, qb, hh), preferred_element_type=F32)
        s_scr[slot, c * CK:(c + 1) * CK, :] = s
        for r in range(CK // 8):
            sr = s[r * 8:(r + 1) * 8]
            m8 = sr if m8 is None else jnp.maximum(m8, sr)
        return m8, s

    def attend(cur, nxt, slot, m8, never, side_work):
        g, _, hh = cur
        mb = jnp.broadcast_to(jnp.max(m8, axis=0, keepdims=True), (8, TQ))
        v0 = pl.multiple_of(g * 64 + hh * (DA // 2), DA // 2)
        m_next = l8 = acc = None
        s_next = []
        for t in range(NC + SKEW):
            if t < NC:
                m_next, s = qk_chunk(nxt, t, 1 - slot, m_next)
                s_next.append(s)
            c = t - SKEW
            if c >= 0:
                ps = [None] * (CK // 8)
                mc = mb
                dep = min(t - DEPLAG, NC - DEPEND)
                for r in reversed(range(CK // 8)):
                    n = CK // 8 - 1 - r
                    if dep >= DEPMIN and n % FINE == 0:
                        mc = jnp.where(never, s_next[dep][(n * DEPMUL // 16) * 8:(n * DEPMUL // 16 + 1) * 8], mb)
                    p = jnp.exp2(
                        s_scr[slot, c * CK + r * 8:c * CK + (r + 1) * 8, :] - mc)
                    ps[r] = p
                    l8 = p if l8 is None else l8 + p
                kb, kt = divmod(c * CK, TQ)
                vt = _b16(vt_u[kb, pl.ds(v0, DA // 2), kt:kt + CK])
                oc = jnp.dot(vt, jnp.concatenate(ps, axis=0).astype(BF16),
                             preferred_element_type=F32)
                acc = oc if acc is None else acc + oc
            if t < NC:
                side_work(hh * NC + t, s)
        return m_next, acc, l8

    def flush(g, qb):
        o = jnp.concatenate(
            [ot_scr[hh] / jnp.sum(l_scr[hh], axis=0, keepdims=True) for hh in range(HPG)],
            axis=0)
        oa_u[g, pl.ds(pl.multiple_of(qb * (TQ // 2), TQ // 2), TQ // 2), :] = (
            _words(o.astype(BF16).T))

    NI = NGA * NQ
    DCH = D // NI
    units = [(n * NST, dst, half, j)
             for n, dst in enumerate((wq_u, wk_u, wv_u))
             for half in range(DCH // 16) for j in range(HB // 2)]

    def relayout(it, base, dst, half, j):
        n = DCH * (HB // 2)
        blk = w_st.at[pl.ds(pl.multiple_of(base + it * n, n), n), :]
        rows = pl.ds(pl.multiple_of(it * (DCH // 2) + half * 8, 8), 8)
        a = blk[pl.ds(half * 16 * (HB // 2) + j, 16, stride=HB // 2), :]
        dst[2 * j, rows, :] = _words(pltpu.bitcast(a << 16, F32).astype(BF16))
        dst[2 * j + 1, rows, :] = _words(
            pltpu.bitcast(a & np.uint32(0xFFFF0000), F32).astype(BF16))

    m8 = None
    for c in range(NC):
        m8, _ = qk_chunk((0, 0, 0), c, 0, m8)
    ot_scr[...] = jnp.zeros(ot_scr.shape, F32)
    l_scr[...] = jnp.ones(l_scr.shape, F32)

    def attn_body(it, m8):
        g, qb = lax.div(it, NQ), lax.rem(it, NQ)
        itn = jnp.minimum(it + 1, NI - 1)
        itp = jnp.maximum(it - 1, 0)
        never = jnp.full((8, TQ), it, jnp.int32) < 0

        def side_work(n, s):
            if n == FLUSH_AT:
                flush(lax.div(itp, NQ), lax.rem(itp, NQ))
            total = HPG * NC
            w_st[3 * NST:, :] = pltpu.bitcast(s[:8, :128], U32)
            for u in units[n * len(units) // total:(n + 1) * len(units) // total]:
                relayout(it, *u)

        for hh in range(HPG):
            nxt = ((g, qb, hh + 1) if hh + 1 < HPG
                   else (lax.div(itn, NQ), lax.rem(itn, NQ), 0))
            m8, acc, l8 = attend((g, qb, hh), nxt, hh % 2, m8, never, side_work)
            ot_scr[hh] = acc
            l_scr[hh] = l8
        return m8

    lax.fori_loop(0, NI, attn_body, m8)
    flush(NGA - 1, NQ - 1)

    row = lax.broadcasted_iota(jnp.int32, (L, L), 0)
    col = lax.broadcasted_iota(jnp.int32, (L, L), 1)
    mask = (row < M) | (row >= col)
    scale = DB ** -0.5
    NG = HB // GB

    def out_copy(s):
        rows = pl.ds(pl.multiple_of(s * seg, seg), seg)
        return pltpu.make_async_copy(out_v.at[rows], out_hbm.at[0, rows], sem_o)

    def wcat(ref, g):
        return jnp.concatenate([_b16(ref[g * GB + i]) for i in range(GB)], axis=1)

    def seg_body(s, mem):
        @pl.when(s > 0)
        def _():
            out_copy(s - 1).start()

        r0 = pl.multiple_of(s * (seg // 2), seg // 2)
        xs = _b16(x_u[pl.ds(r0, seg // 2), :]).astype(F32)
        h = jnp.concatenate([mem, xs], axis=0)
        Q, K, V, P, O = {}, {}, {}, {}, {}
        acc = [None]

        def proj(dst, ref, g):
            dst[g] = jnp.dot(h, wcat(ref, g), preferred_element_type=F32)

        def scores(g):
            q, k = Q.pop(g), K.pop(g)
            P[g] = []
            for i in range(GB):
                sl = slice(i * DB, (i + 1) * DB)
                sc = lax.dot_general(q[:, sl], k[:, sl].astype(BF16), NT_DIMS,
                                     preferred_element_type=F32) * scale
                sc = jnp.where(mask, sc, -1000000000.0)
                e = jnp.exp(sc - jnp.max(sc, axis=-1, keepdims=True))
                P[g].append((e, jnp.sum(e, axis=-1, keepdims=True)))

        def mix(g):
            v, ps = V.pop(g), P.pop(g)
            outs = []
            for i in range(GB):
                e, l = ps[i]
                o = jnp.dot(e, v[:, i * DB:(i + 1) * DB].astype(BF16),
                            preferred_element_type=F32)
                outs.append(o / l)
            O[g] = jnp.concatenate(outs, axis=1)

        def outp(g):
            n = GB * DB // 2
            r = jnp.dot(O.pop(g), _b16(wob_u[g * n:(g + 1) * n, :]),
                        preferred_element_type=F32)
            acc[0] = r if acc[0] is None else acc[0] + r

        for t in range(NG + 1):
            if t < NG:
                proj(Q, wq_u, t)
                proj(K, wk_u, t)
            else:
                proj(V, wv_u, 0)
            if t >= 1:
                scores(t - 1)
        lag = 3
        for t in range(1, NG + lag):
            if t < NG:
                proj(V, wv_u, t)
            if t - 1 < NG:
                mix(t - 1)
            if t >= lag:
                outp(t - lag)

        oa = jnp.concatenate(
            [_b16(oa_u[g, pl.ds(r0, seg // 2), :]) for g in range(NGA)], axis=1)
        a = jnp.dot(oa, _b16(wo_u[...]), preferred_element_type=F32)
        gate = jax.nn.sigmoid(
            jnp.sum(xs * gate_ref[...].astype(F32), axis=-1, keepdims=True))
        res = gate * a + (1.0 - gate) * acc[0][M:]
        out_v[pl.ds(pl.multiple_of(s * seg, seg), seg), :] = res.astype(BF16)
        return acc[0][:M].astype(BF16).astype(F32)

    lax.fori_loop(0, NS, seg_body, mem0_ref[0].astype(F32))
    out_copy(NS - 1).start()
    pltpu.make_async_copy(out_v, out_hbm.at[0], sem_o).wait()


@functools.partial(jax.jit, static_argnames=("B_seg_len",))
def pallas_gated_mix__softmax_full_mha__memory_aug_recurrent_mem_tr__prompt_kernel(
    A_x: jax.Array,
    A_wqkv: jax.Array,
    A_wo: jax.Array,
    B_x: jax.Array,
    B_mem0: jax.Array,
    B_Wq: jax.Array,
    B_Wk: jax.Array,
    B_Wv: jax.Array,
    B_Wo: jax.Array,
    B_seg_len: int,
    gate_w: jax.Array,
):
    del B_x
    B, S, D = A_x.shape
    _, HB, DB = B_Wq.shape
    seg = int(B_seg_len)
    assert B == 1 and S % TQ == 0 and D % CN == 0 and S % seg == 0 and seg % 16 == 0
    assert DB == 128 and HB % GB == 0 and B_mem0.shape[1] % 8 == 0

    hbm = pl.BlockSpec(memory_space=pl.ANY)
    vmem = pl.BlockSpec(memory_space=pltpu.VMEM)
    per_head = pltpu.VMEM((HB, D // 2, DB), U32)
    scratch = [
        pltpu.VMEM((S // 2, D), U32),
        pltpu.VMEM((3 * D // CN, D // 2, CN), U32),
        pltpu.VMEM((D // 2, D), U32),
        pltpu.VMEM((HB * DB // 2, D), U32),
        pltpu.VMEM((3 * D * HB // 2 + 8, DB), U32),
        per_head, per_head, per_head,
        pltpu.VMEM((D // 128, S // 2, 128), U32),
        pltpu.VMEM((S // TQ, D // 2, TQ), U32),
        pltpu.VMEM((S // TQ, D // 2, TQ), U32),
        pltpu.VMEM((2, S, TQ), F32),
        pltpu.VMEM((128 * HA // D, D // HA, TQ), F32),
        pltpu.VMEM((128 * HA // D, 8, TQ), F32),
        pltpu.VMEM((D // 128, S // 2, 128), U32),
        pltpu.VMEM((S, D), BF16),
        pltpu.SemaphoreType.DMA((S // TQ,)),
        pltpu.SemaphoreType.DMA((3 * D // CN,)),
        pltpu.SemaphoreType.DMA((5,)),
        pltpu.SemaphoreType.DMA,
    ]
    return pl.pallas_call(
        functools.partial(_kernel, seg=seg),
        out_shape=jax.ShapeDtypeStruct((B, S, D), A_x.dtype),
        in_specs=[hbm, hbm, hbm, vmem, hbm, hbm, hbm, hbm, vmem],
        out_specs=hbm,
        scratch_shapes=scratch,
        compiler_params=pltpu.CompilerParams(vmem_limit_bytes=120 * 2**20),
    )(
        A_x.reshape(S, D), A_wqkv, A_wo, B_mem0,
        B_Wq.reshape(D * HB, DB), B_Wk.reshape(D * HB, DB), B_Wv.reshape(D * HB, DB),
        B_Wo.reshape(HB * DB, D), gate_w.reshape(1, D),
    )
```

```python
import functools

import jax
import jax.numpy as jnp
import numpy as np
from jax import lax
from jax.experimental import pallas as pl
from jax.experimental.pallas import tpu as pltpu

BF16 = jnp.bfloat16
F32 = jnp.float32
U32 = jnp.uint32
LOG2E = float(np.log2(np.e))
NT_DIMS = (((1,), (1,)), ((), ()))

TQ = 512
CN = 512
CK = 128
HA = 32
GB = 4
SKEW = 1
FLUSH_AT = 4
PRE = 2
STEP = 2
UA = 2
UB = 2
DEPLAG = 1
DEPEND = 2
DEPMIN = 0
FINE = 2
DEPMUL = 16


def _b16(words):
    return pltpu.bitcast(words, BF16)


def _words(x):
    return pltpu.bitcast(x, U32)


def _kernel(
    x_hbm, wqkv_hbm, wo_hbm, mem0_ref, wq_hbm, wk_hbm, wv_hbm, wob_hbm, gate_ref,
    out_hbm,
    x_u, wqkv_u, wo_u, wob_u, w_st, wq_u, wk_u, wv_u,
    k_u, qt_u, vt_u, s_scr, ot_scr, l_scr, oa_u, out_v,
    sem_x, sem_w, sem_b, sem_o,
    *, seg,
):
    S2, D = x_u.shape
    S = 2 * S2
    DA = D // HA
    NQ = S // TQ
    NGA = D // 128
    HPG = 128 // DA
    NC = S // CK
    NCB = D // CN
    HB, _, DB = wq_u.shape
    M = mem0_ref.shape[1]
    L = M + seg
    NS = S // seg

    def x_copy(i):
        rows = pl.ds(i * (TQ // 2), TQ // 2)
        return pltpu.make_async_copy(
            x_hbm.bitcast(U32).at[rows], x_u.at[rows], sem_x.at[i])

    def w_copy(j):
        return pltpu.make_async_copy(
            wqkv_hbm.bitcast(U32).at[:, pl.ds(j * CN, CN)], wqkv_u.at[j], sem_w.at[j])

    NST = D * HB // 2
    late_copies = [
        pltpu.make_async_copy(src.bitcast(U32), dst, sem_b.at[n])
        for n, (src, dst) in enumerate((
            (wq_hbm, w_st.at[pl.ds(0, NST)]), (wk_hbm, w_st.at[pl.ds(NST, NST)]),
            (wv_hbm, w_st.at[pl.ds(2 * NST, NST)]), (wob_hbm, wob_u), (wo_hbm, wo_u)))
    ]
    queue = ([x_copy(0)] + [w_copy(j) for j in range(3 * NCB)]
             + [x_copy(i) for i in range(1, NQ)] + late_copies)

    def start_copies(n):
        for _ in range(min(n, len(queue))):
            queue.pop(0).start()

    start_copies(PRE)

    qscale = (DA ** -0.5) * LOG2E

    def proj_rows(i, first):
        x_copy(i).wait()
        r0 = i * (TQ // 2) if first else pl.multiple_of(i * (TQ // 2), TQ // 2)
        for j in range(3 * NCB):
            if first:
                w_copy(j).wait()
                start_copies(STEP)
            r = jnp.dot(_b16(x_u[pl.ds(r0, TQ // 2), :]), _b16(wqkv_u[j]),
                        preferred_element_type=F32)
            which, jb = divmod(j, NCB)
            rows = slice(jb * (CN // 2), (jb + 1) * (CN // 2))
            if which == 0:
                qt_u[i, rows, :] = _words((r * qscale).astype(BF16).T)
            elif which == 1:
                rb = _words(r.astype(BF16))
                for t in range(CN // 128):
                    k_u[jb * (CN // 128) + t, pl.ds(r0, TQ // 2), :] = (
                        rb[:, t * 128:(t + 1) * 128])
            else:
                vt_u[i, rows, :] = _words(r.astype(BF16).T)

    proj_rows(0, True)
    start_copies(len(queue))

    @pl.loop(1, NQ)
    def _(i):
        proj_rows(i, False)

    for cp in late_copies:
        cp.wait()

    def masked_qt(g, qb, hh):
        r0 = pl.multiple_of(g * 64 + hh * (DA // 2), DA // 2)
        parts = []
        if hh > 0:
            parts.append(jnp.zeros((hh * (DA // 2), TQ), U32))
        parts.append(qt_u[qb, pl.ds(r0, DA // 2), :])
        if hh < HPG - 1:
            parts.append(jnp.zeros(((HPG - 1 - hh) * (DA // 2), TQ), U32))
        return _b16(jnp.concatenate(parts, axis=0))

    def qk_chunk(item, c, slot, m8):
        g, qb, hh = item
        s = jnp.dot(_b16(k_u[g, c * (CK // 2):(c + 1) * (CK // 2), :]),
                    masked_qt(g, qb, hh), preferred_element_type=F32)
        s_scr[slot, c * CK:(c + 1) * CK, :] = s
        for r in range(CK // 8):
            sr = s[r * 8:(r + 1) * 8]
            m8 = sr if m8 is None else jnp.maximum(m8, sr)
        return m8, s

    def attend(cur, nxt, slot, m8, never, side_work):
        g, _, hh = cur
        mb = jnp.broadcast_to(jnp.max(m8, axis=0, keepdims=True), (8, TQ))
        v0 = pl.multiple_of(g * 64 + hh * (DA // 2), DA // 2)
        m_next = l8 = acc = None
        s_next = []
        for t in range(NC + SKEW):
            if t < NC:
                m_next, s = qk_chunk(nxt, t, 1 - slot, m_next)
                s_next.append(s)
            c = t - SKEW
            if c >= 0:
                ps = [None] * (CK // 8)
                mc = mb
                dep = min(t - DEPLAG, NC - DEPEND)
                for r in reversed(range(CK // 8)):
                    n = CK // 8 - 1 - r
                    if dep >= DEPMIN and n % FINE == 0:
                        mc = jnp.where(never, s_next[dep][(n * DEPMUL // 16) * 8:(n * DEPMUL // 16 + 1) * 8], mb)
                    p = jnp.exp2(
                        s_scr[slot, c * CK + r * 8:c * CK + (r + 1) * 8, :] - mc)
                    ps[r] = p
                    l8 = p if l8 is None else l8 + p
                kb, kt = divmod(c * CK, TQ)
                vt = _b16(vt_u[kb, pl.ds(v0, DA // 2), kt:kt + CK])
                oc = jnp.dot(vt, jnp.concatenate(ps, axis=0).astype(BF16),
                             preferred_element_type=F32)
                acc = oc if acc is None else acc + oc
            if t < NC:
                side_work(hh * NC + t, s)
        return m_next, acc, l8

    def flush(g, qb):
        o = jnp.concatenate(
            [ot_scr[hh] / jnp.sum(l_scr[hh], axis=0, keepdims=True) for hh in range(HPG)],
            axis=0)
        oa_u[g, pl.ds(pl.multiple_of(qb * (TQ // 2), TQ // 2), TQ // 2), :] = (
            _words(o.astype(BF16).T))

    NI = NGA * NQ
    DCH = D // NI
    units = [(n * NST, dst, half, j)
             for n, dst in enumerate((wq_u, wk_u, wv_u))
             for half in range(DCH // 16) for j in range(HB // 2)]

    def relayout(it, base, dst, half, j):
        n = DCH * (HB // 2)
        blk = w_st.at[pl.ds(pl.multiple_of(base + it * n, n), n), :]
        rows = pl.ds(pl.multiple_of(it * (DCH // 2) + half * 8, 8), 8)
        a = blk[pl.ds(half * 16 * (HB // 2) + j, 16, stride=HB // 2), :]
        dst[2 * j, rows, :] = _words(pltpu.bitcast(a << 16, F32).astype(BF16))
        dst[2 * j + 1, rows, :] = _words(
            pltpu.bitcast(a & np.uint32(0xFFFF0000), F32).astype(BF16))

    m8 = None
    for c in range(NC):
        m8, _ = qk_chunk((0, 0, 0), c, 0, m8)
    ot_scr[...] = jnp.zeros(ot_scr.shape, F32)
    l_scr[...] = jnp.ones(l_scr.shape, F32)

    def attn_body(it, m8):
        g, qb = lax.div(it, NQ), lax.rem(it, NQ)
        itn = jnp.minimum(it + 1, NI - 1)
        itp = jnp.maximum(it - 1, 0)
        never = jnp.full((8, TQ), it, jnp.int32) < 0

        def side_work(n, s):
            if n == FLUSH_AT:
                flush(lax.div(itp, NQ), lax.rem(itp, NQ))
            total = HPG * NC
            w_st[3 * NST:, :] = pltpu.bitcast(s[:8, :128], U32)
            for u in units[n * len(units) // total:(n + 1) * len(units) // total]:
                relayout(it, *u)

        for hh in range(HPG):
            nxt = ((g, qb, hh + 1) if hh + 1 < HPG
                   else (lax.div(itn, NQ), lax.rem(itn, NQ), 0))
            m8, acc, l8 = attend((g, qb, hh), nxt, hh % 2, m8, never, side_work)
            ot_scr[hh] = acc
            l_scr[hh] = l8
        return m8

    def attn_bodies(n, m8):
        for u in range(UA):
            m8 = attn_body(n * UA + u, m8)
        return m8

    lax.fori_loop(0, NI // UA, attn_bodies, m8)
    flush(NGA - 1, NQ - 1)

    row = lax.broadcasted_iota(jnp.int32, (L, L), 0)
    col = lax.broadcasted_iota(jnp.int32, (L, L), 1)
    mask = (row < M) | (row >= col)
    scale = DB ** -0.5
    NG = HB // GB

    def out_copy(n):
        rows = pl.ds(pl.multiple_of(n * (UB * seg), UB * seg), UB * seg)
        return pltpu.make_async_copy(out_v.at[rows], out_hbm.at[0, rows], sem_o)

    def wcat(ref, g):
        return jnp.concatenate([_b16(ref[g * GB + i]) for i in range(GB)], axis=1)

    gate_w = gate_ref[...].astype(F32).reshape(1, D)

    def seg_body(s, mem):
        r0 = pl.multiple_of(s * (seg // 2), seg // 2)
        xs = _b16(x_u[pl.ds(r0, seg // 2), :]).astype(F32)
        h = jnp.concatenate([mem, xs], axis=0)
        Q, K, V, P, O = {}, {}, {}, {}, {}
        acc = [None]

        def proj(dst, ref, g):
            dst[g] = jnp.dot(h, wcat(ref, g), preferred_element_type=F32)

        def scores(g):
            q, k = Q.pop(g), K.pop(g)
            P[g] = []
            for i in range(GB):
                sl = slice(i * DB, (i + 1) * DB)
                sc = lax.dot_general(q[:, sl], k[:, sl].astype(BF16), NT_DIMS,
                                     preferred_element_type=F32) * scale
                sc = jnp.where(mask, sc, -1000000000.0)
                e = jnp.exp(sc - jnp.max(sc, axis=-1, keepdims=True))
                P[g].append((e, jnp.sum(e, axis=-1, keepdims=True)))

        def mix(g):
            v, ps = V.pop(g), P.pop(g)
            outs = []
            for i in range(GB):
                e, l = ps[i]
                o = jnp.dot(e, v[:, i * DB:(i + 1) * DB].astype(BF16),
                            preferred_element_type=F32)
                outs.append(o / l)
            O[g] = jnp.concatenate(outs, axis=1)

        def outp(g):
            n = GB * DB // 2
            r = jnp.dot(O.pop(g), _b16(wob_u[g * n:(g + 1) * n, :]),
                        preferred_element_type=F32)
            acc[0] = r if acc[0] is None else acc[0] + r

        for t in range(NG + 1):
            if t < NG:
                proj(Q, wq_u, t)
                proj(K, wk_u, t)
            else:
                proj(V, wv_u, 0)
            if t >= 1:
                scores(t - 1)
        lag = 3
        for t in range(1, NG + lag):
            if t < NG:
                proj(V, wv_u, t)
            if t - 1 < NG:
                mix(t - 1)
            if t >= lag:
                outp(t - lag)

        oa = jnp.concatenate(
            [_b16(oa_u[g, pl.ds(r0, seg // 2), :]) for g in range(NGA)], axis=1)
        a = jnp.dot(oa, _b16(wo_u[...]), preferred_element_type=F32)
        gate = jax.nn.sigmoid(
            jnp.sum(xs * gate_w, axis=-1, keepdims=True))
        res = gate * a + (1.0 - gate) * acc[0][M:]
        out_v[pl.ds(pl.multiple_of(s * seg, seg), seg), :] = res.astype(BF16)
        return acc[0][:M].astype(BF16).astype(F32)

    def seg_bodies(n, mem):
        @pl.when(n > 0)
        def _():
            out_copy(n - 1).start()

        for u in range(UB):
            mem = seg_body(n * UB + u, mem)
        return mem

    lax.fori_loop(0, NS // UB, seg_bodies, mem0_ref[0].astype(F32))
    out_copy(NS // UB - 1).start()
    pltpu.make_async_copy(out_v, out_hbm.at[0], sem_o).wait()


@functools.partial(jax.jit, static_argnames=("B_seg_len",))
def pallas_gated_mix__softmax_full_mha__memory_aug_recurrent_mem_tr__prompt_kernel(
    A_x: jax.Array,
    A_wqkv: jax.Array,
    A_wo: jax.Array,
    B_x: jax.Array,
    B_mem0: jax.Array,
    B_Wq: jax.Array,
    B_Wk: jax.Array,
    B_Wv: jax.Array,
    B_Wo: jax.Array,
    B_seg_len: int,
    gate_w: jax.Array,
):
    del B_x
    B, S, D = A_x.shape
    _, HB, DB = B_Wq.shape
    seg = int(B_seg_len)
    assert B == 1 and S % TQ == 0 and D % CN == 0 and S % seg == 0 and seg % 16 == 0
    assert DB == 128 and HB % GB == 0 and B_mem0.shape[1] % 8 == 0

    hbm = pl.BlockSpec(memory_space=pl.ANY)
    vmem = pl.BlockSpec(memory_space=pltpu.VMEM)
    per_head = pltpu.VMEM((HB, D // 2, DB), U32)
    scratch = [
        pltpu.VMEM((S // 2, D), U32),
        pltpu.VMEM((3 * D // CN, D // 2, CN), U32),
        pltpu.VMEM((D // 2, D), U32),
        pltpu.VMEM((HB * DB // 2, D), U32),
        pltpu.VMEM((3 * D * HB // 2 + 8, DB), U32),
        per_head, per_head, per_head,
        pltpu.VMEM((D // 128, S // 2, 128), U32),
        pltpu.VMEM((S // TQ, D // 2, TQ), U32),
        pltpu.VMEM((S // TQ, D // 2, TQ), U32),
        pltpu.VMEM((2, S, TQ), F32),
        pltpu.VMEM((128 * HA // D, D // HA, TQ), F32),
        pltpu.VMEM((128 * HA // D, 8, TQ), F32),
        pltpu.VMEM((D // 128, S // 2, 128), U32),
        pltpu.VMEM((S, D), BF16),
        pltpu.SemaphoreType.DMA((S // TQ,)),
        pltpu.SemaphoreType.DMA((3 * D // CN,)),
        pltpu.SemaphoreType.DMA((5,)),
        pltpu.SemaphoreType.DMA,
    ]
    return pl.pallas_call(
        functools.partial(_kernel, seg=seg),
        out_shape=jax.ShapeDtypeStruct((B, S, D), A_x.dtype),
        in_specs=[hbm, hbm, hbm, vmem, hbm, hbm, hbm, hbm, vmem],
        out_specs=hbm,
        scratch_shapes=scratch,
        compiler_params=pltpu.CompilerParams(vmem_limit_bytes=120 * 2**20),
    )(
        A_x.reshape(S, D), A_wqkv, A_wo, B_mem0,
        B_Wq.reshape(D * HB, DB), B_Wk.reshape(D * HB, DB), B_Wv.reshape(D * HB, DB),
        B_Wo.reshape(HB * DB, D), gate_w,
    )
```

```python
import functools

import jax
import jax.numpy as jnp
import numpy as np
from jax import lax
from jax.experimental import pallas as pl
from jax.experimental.pallas import tpu as pltpu

BF16 = jnp.bfloat16
F32 = jnp.float32
U32 = jnp.uint32
LOG2E = float(np.log2(np.e))
NT_DIMS = (((1,), (1,)), ((), ()))

TQ = 512
CN = 512
CK = 128
HA = 32
GB = 4
UA = 2
UB = 2
SPARE = 16


def _b16(words):
    return pltpu.bitcast(words, BF16)


def _words(x):
    return pltpu.bitcast(x, U32)


def _kernel(
    x_hbm, wqkv_hbm, wo_hbm, mem0_ref, wq_hbm, wk_hbm, wv_hbm, wob_hbm, gate_ref,
    out_hbm,
    x_u, wqkv_u, wo_u, wob_u, w_st, wq_u, wk_u, wv_u,
    k_u, qt_u, vt_u, s_scr, ot_scr, l_scr, oa_u, out_v,
    sem_x, sem_w, sem_b, sem_o,
    *, seg,
):
    S2, D = x_u.shape
    S = 2 * S2
    DA = D // HA
    NQ = S // TQ
    NGA = D // 128
    HPG = 128 // DA
    NC = S // CK
    NCB = D // CN
    HB, _, DB = wq_u.shape
    M = mem0_ref.shape[1]
    L = M + seg
    NS = S // seg

    def x_copy(i):
        rows = pl.ds(i * (TQ // 2), TQ // 2)
        return pltpu.make_async_copy(
            x_hbm.bitcast(U32).at[rows], x_u.at[rows], sem_x.at[i])

    def w_copy(j):
        return pltpu.make_async_copy(
            wqkv_hbm.bitcast(U32).at[:, pl.ds(j * CN, CN)], wqkv_u.at[j], sem_w.at[j])

    NST = D * HB // 2
    late_copies = [
        pltpu.make_async_copy(src.bitcast(U32), dst, sem_b.at[n])
        for n, (src, dst) in enumerate((
            (wq_hbm, w_st.at[pl.ds(0, NST)]), (wk_hbm, w_st.at[pl.ds(NST, NST)]),
            (wv_hbm, w_st.at[pl.ds(2 * NST, NST)]), (wob_hbm, wob_u), (wo_hbm, wo_u)))
    ]
    queue = ([x_copy(0)] + [w_copy(j) for j in range(3 * NCB)]
             + [x_copy(i) for i in range(1, NQ)] + late_copies)

    def start_copies(n):
        for _ in range(min(n, len(queue))):
            queue.pop(0).start()

    start_copies(2)

    qscale = (DA ** -0.5) * LOG2E

    def proj_rows(i, first):
        x_copy(i).wait()
        r0 = i * (TQ // 2) if first else pl.multiple_of(i * (TQ // 2), TQ // 2)
        for j in range(3 * NCB):
            if first and j < 3:
                w_copy(j).wait()
                start_copies(4 if j == 0 else 1)
            elif first and j == 3:
                for jj in range(j, 3 * NCB):
                    w_copy(jj).wait()
                start_copies(len(queue))
            r = jnp.dot(_b16(x_u[pl.ds(r0, TQ // 2), :]), _b16(wqkv_u[j]),
                        preferred_element_type=F32)
            which, jb = divmod(j, NCB)
            rows = slice(jb * (CN // 2), (jb + 1) * (CN // 2))
            if which == 0:
                qt_u[i, rows, :] = _words((r * qscale).astype(BF16).T)
            elif which == 1:
                rb = _words(r.astype(BF16))
                for t in range(CN // 128):
                    k_u[jb * (CN // 128) + t, pl.ds(r0, TQ // 2), :] = (
                        rb[:, t * 128:(t + 1) * 128])
            else:
                vt_u[i, rows, :] = _words(r.astype(BF16).T)

    proj_rows(0, True)
    assert not queue

    @pl.loop(1, NQ)
    def _(i):
        proj_rows(i, False)

    for cp in late_copies:
        cp.wait()

    def masked_qt(g, qb, hh):
        r0 = pl.multiple_of(g * 64 + hh * (DA // 2), DA // 2)
        parts = []
        if hh > 0:
            parts.append(jnp.zeros((hh * (DA // 2), TQ), U32))
        parts.append(qt_u[qb, pl.ds(r0, DA // 2), :])
        if hh < HPG - 1:
            parts.append(jnp.zeros(((HPG - 1 - hh) * (DA // 2), TQ), U32))
        return _b16(jnp.concatenate(parts, axis=0))

    def qk_chunk(item, c, slot, m8):
        g, qb, hh = item
        s = jnp.dot(_b16(k_u[g, c * (CK // 2):(c + 1) * (CK // 2), :]),
                    masked_qt(g, qb, hh), preferred_element_type=F32)
        s_scr[slot, c * CK:(c + 1) * CK, :] = s
        for r in range(CK // 8):
            sr = s[r * 8:(r + 1) * 8]
            m8 = sr if m8 is None else jnp.maximum(m8, sr)
        return m8, s

    def attend(cur, nxt, slot, m8, never, side_work):
        g, _, hh = cur
        mb = jnp.broadcast_to(jnp.max(m8, axis=0, keepdims=True), (8, TQ))
        v0 = pl.multiple_of(g * 64 + hh * (DA // 2), DA // 2)
        m_next = l8 = acc = None
        s_next = []
        for t in range(NC + 1):
            if t < NC:
                m_next, s = qk_chunk(nxt, t, 1 - slot, m_next)
                s_next.append(s)
            if t > 0:
                c = t - 1
                pace = s_next[min(c, NC - 2)]
                ps = [None] * (CK // 8)
                for n in range(CK // 8):
                    r = CK // 8 - 1 - n
                    if n % 2 == 0:
                        mc = jnp.where(never, pace[n * 8:(n + 1) * 8], mb)
                    ps[r] = jnp.exp2(
                        s_scr[slot, c * CK + r * 8:c * CK + (r + 1) * 8, :] - mc)
                    l8 = ps[r] if l8 is None else l8 + ps[r]
                kb, kt = divmod(c * CK, TQ)
                vt = _b16(vt_u[kb, pl.ds(v0, DA // 2), kt:kt + CK])
                oc = jnp.dot(vt, jnp.concatenate(ps, axis=0).astype(BF16),
                             preferred_element_type=F32)
                acc = oc if acc is None else acc + oc
            if t < NC:
                side_work(hh * NC + t, s)
        return m_next, acc, l8

    def flush(g, qb):
        o = jnp.concatenate(
            [ot_scr[hh] / jnp.sum(l_scr[hh], axis=0, keepdims=True) for hh in range(HPG)],
            axis=0)
        oa_u[g, pl.ds(pl.multiple_of(qb * (TQ // 2), TQ // 2), TQ // 2), :] = (
            _words(o.astype(BF16).T))

    NI = NGA * NQ
    DCH = D // NI
    units = [(n * NST, dst, half, j)
             for n, dst in enumerate((wq_u, wk_u, wv_u))
             for half in range(DCH // 16) for j in range(HB // 2)]

    def relayout(it, base, dst, half, j):
        n = DCH * (HB // 2)
        blk = w_st.at[pl.ds(pl.multiple_of(base + it * n, n), n + SPARE), :]
        rows = pl.ds(pl.multiple_of(it * (DCH // 2) + half * 8, 8), 8)
        a = blk[pl.ds(half * 16 * (HB // 2) + j, 16, stride=HB // 2), :]
        dst[2 * j, rows, :] = _words(pltpu.bitcast(a << 16, F32).astype(BF16))
        dst[2 * j + 1, rows, :] = _words(
            pltpu.bitcast(a & np.uint32(0xFFFF0000), F32).astype(BF16))

    m8 = None
    for c in range(NC):
        m8, _ = qk_chunk((0, 0, 0), c, 0, m8)
    ot_scr[...] = jnp.zeros(ot_scr.shape, F32)
    l_scr[...] = jnp.ones(l_scr.shape, F32)

    def attn_body(it, m8):
        g, qb = lax.div(it, NQ), lax.rem(it, NQ)
        itn = jnp.minimum(it + 1, NI - 1)
        itp = jnp.maximum(it - 1, 0)
        never = jnp.full((8, TQ), it, jnp.int32) < 0

        def side_work(n, s):
            if n == 4:
                flush(lax.div(itp, NQ), lax.rem(itp, NQ))
            total = HPG * NC
            w_st[3 * NST:3 * NST + 8, :] = pltpu.bitcast(s[:8, :128], U32)
            for u in units[n * len(units) // total:(n + 1) * len(units) // total]:
                relayout(it, *u)

        for hh in range(HPG):
            nxt = ((g, qb, hh + 1) if hh + 1 < HPG
                   else (lax.div(itn, NQ), lax.rem(itn, NQ), 0))
            m8, acc, l8 = attend((g, qb, hh), nxt, hh % 2, m8, never, side_work)
            ot_scr[hh] = acc
            l_scr[hh] = l8
        return m8

    def attn_bodies(n, m8):
        for u in range(UA):
            m8 = attn_body(n * UA + u, m8)
        return m8

    lax.fori_loop(0, NI // UA, attn_bodies, m8)
    flush(NGA - 1, NQ - 1)

    row = lax.broadcasted_iota(jnp.int32, (L, L), 0)
    col = lax.broadcasted_iota(jnp.int32, (L, L), 1)
    mask = (row < M) | (row >= col)
    scale = DB ** -0.5
    NG = HB // GB

    def out_copy(n):
        rows = pl.ds(pl.multiple_of(n * (UB * seg), UB * seg), UB * seg)
        return pltpu.make_async_copy(out_v.at[rows], out_hbm.at[0, rows], sem_o)

    def wcat(ref, g):
        return jnp.concatenate([_b16(ref[g * GB + i]) for i in range(GB)], axis=1)

    gate_w = gate_ref[...].astype(F32).reshape(1, D)

    def seg_body(s, mem):
        r0 = pl.multiple_of(s * (seg // 2), seg // 2)
        xs = _b16(x_u[pl.ds(r0, seg // 2), :]).astype(F32)
        h = jnp.concatenate([mem, xs], axis=0)
        Q, K, V, P, O = {}, {}, {}, {}, {}
        acc = [None]

        def proj(dst, ref, g):
            dst[g] = jnp.dot(h, wcat(ref, g), preferred_element_type=F32)

        def scores(g):
            q, k = Q.pop(g), K.pop(g)
            P[g] = []
            for i in range(GB):
                sl = slice(i * DB, (i + 1) * DB)
                sc = lax.dot_general(q[:, sl], k[:, sl].astype(BF16), NT_DIMS,
                                     preferred_element_type=F32) * scale
                sc = jnp.where(mask, sc, -1000000000.0)
                e = jnp.exp(sc - jnp.max(sc, axis=-1, keepdims=True))
                P[g].append((e, jnp.sum(e, axis=-1, keepdims=True)))

        def mix(g):
            v, ps = V.pop(g), P.pop(g)
            outs = []
            for i in range(GB):
                e, l = ps[i]
                o = jnp.dot(e, v[:, i * DB:(i + 1) * DB].astype(BF16),
                            preferred_element_type=F32)
                outs.append(o / l)
            O[g] = jnp.concatenate(outs, axis=1)

        def outp(g):
            n = GB * DB // 2
            r = jnp.dot(O.pop(g), _b16(wob_u[g * n:(g + 1) * n, :]),
                        preferred_element_type=F32)
            acc[0] = r if acc[0] is None else acc[0] + r

        for t in range(NG + 1):
            if t < NG:
                proj(Q, wq_u, t)
                proj(K, wk_u, t)
            else:
                proj(V, wv_u, 0)
            if t >= 1:
                scores(t - 1)
        for t in range(1, NG + 2):
            if t < NG:
                proj(V, wv_u, t)
            if t <= NG:
                mix(t - 1)
            if t >= 2:
                outp(t - 2)

        oa = jnp.concatenate(
            [_b16(oa_u[g, pl.ds(r0, seg // 2), :]) for g in range(NGA)], axis=1)
        a = jnp.dot(oa, _b16(wo_u[...]), preferred_element_type=F32)
        gate = jax.nn.sigmoid(jnp.sum(xs * gate_w, axis=-1, keepdims=True))
        res = gate * a + (1.0 - gate) * acc[0][M:]
        out_v[pl.ds(pl.multiple_of(s * seg, seg), seg), :] = res.astype(BF16)
        return acc[0][:M].astype(BF16).astype(F32)

    def seg_bodies(n, mem):
        @pl.when(n > 0)
        def _():
            out_copy(n - 1).start()

        for u in range(UB):
            mem = seg_body(n * UB + u, mem)
        return mem

    lax.fori_loop(0, NS // UB, seg_bodies, mem0_ref[0].astype(F32))
    out_copy(NS // UB - 1).start()
    pltpu.make_async_copy(out_v, out_hbm.at[0], sem_o).wait()


@functools.partial(jax.jit, static_argnames=("B_seg_len",))
def pallas_gated_mix__softmax_full_mha__memory_aug_recurrent_mem_tr__prompt_kernel(
    A_x: jax.Array,
    A_wqkv: jax.Array,
    A_wo: jax.Array,
    B_x: jax.Array,
    B_mem0: jax.Array,
    B_Wq: jax.Array,
    B_Wk: jax.Array,
    B_Wv: jax.Array,
    B_Wo: jax.Array,
    B_seg_len: int,
    gate_w: jax.Array,
):
    del B_x
    B, S, D = A_x.shape
    _, HB, DB = B_Wq.shape
    seg = int(B_seg_len)
    assert B == 1 and S % TQ == 0 and D % CN == 0 and S % seg == 0 and seg % 16 == 0
    assert DB == 128 and HB % GB == 0 and B_mem0.shape[1] % 8 == 0
    assert (S // seg) % UB == 0 and D == 1024

    hbm = pl.BlockSpec(memory_space=pl.ANY)
    vmem = pl.BlockSpec(memory_space=pltpu.VMEM)
    per_head = pltpu.VMEM((HB, D // 2, DB), U32)
    scratch = [
        pltpu.VMEM((S // 2, D), U32),
        pltpu.VMEM((3 * D // CN, D // 2, CN), U32),
        pltpu.VMEM((D // 2, D), U32),
        pltpu.VMEM((HB * DB // 2, D), U32),
        pltpu.VMEM((3 * D * HB // 2 + SPARE, DB), U32),
        per_head, per_head, per_head,
        pltpu.VMEM((D // 128, S // 2, 128), U32),
        pltpu.VMEM((S // TQ, D // 2, TQ), U32),
        pltpu.VMEM((S // TQ, D // 2, TQ), U32),
        pltpu.VMEM((2, S, TQ), F32),
        pltpu.VMEM((128 * HA // D, D // HA, TQ), F32),
        pltpu.VMEM((128 * HA // D, 8, TQ), F32),
        pltpu.VMEM((D // 128, S // 2, 128), U32),
        pltpu.VMEM((S, D), BF16),
        pltpu.SemaphoreType.DMA((S // TQ,)),
        pltpu.SemaphoreType.DMA((3 * D // CN,)),
        pltpu.SemaphoreType.DMA((5,)),
        pltpu.SemaphoreType.DMA,
    ]
    return pl.pallas_call(
        functools.partial(_kernel, seg=seg),
        out_shape=jax.ShapeDtypeStruct((B, S, D), A_x.dtype),
        in_specs=[hbm, hbm, hbm, vmem, hbm, hbm, hbm, hbm, vmem],
        out_specs=hbm,
        scratch_shapes=scratch,
        compiler_params=pltpu.CompilerParams(vmem_limit_bytes=120 * 2**20),
    )(
        A_x.reshape(S, D), A_wqkv, A_wo, B_mem0,
        B_Wq.reshape(D * HB, DB), B_Wk.reshape(D * HB, DB), B_Wv.reshape(D * HB, DB),
        B_Wo.reshape(HB * DB, D), gate_w,
    )
```
